```python
import os as _os
_os.environ.setdefault("JAX_PLATFORMS", "cpu")
import jax
import jax.numpy as jnp

def _softmax(x, axis=-1):
    return jax.nn.softmax(x, axis=axis)
def _gelu(x):
    return jax.nn.gelu(x, approximate=True)
def _silu(x):
    return jax.nn.silu(x)
def _sigmoid(x):
    return jax.nn.sigmoid(x)
def _layernorm(x, axis=-1, eps=1e-5):
    m = jnp.mean(x, axis=axis, keepdims=True)
    v = jnp.var(x, axis=axis, keepdims=True)
    return (x - m) / jnp.sqrt(v + eps)
def _scatter_add(tgt, idx, src, axis=0):
    return tgt.at[idx].add(src)
def _segment_sum(src, seg, n):
    return jax.ops.segment_sum(src, seg, n)
class _Rng:
    def __init__(self, key):
        self._k = key
    def _next(self):
        self._k, sub = jax.random.split(self._k)
        return sub
    def normal(self, shape):
        return jax.random.normal(self._next(), shape, dtype=jnp.bfloat16)
    def randint(self, lo, hi, shape):
        return jax.random.randint(self._next(), shape, lo, hi, dtype=jnp.int32)
    def uniform(self, shape, lo=0.0, hi=1.0):
        return jax.random.uniform(self._next(), shape, jnp.bfloat16, lo, hi)
    def permutation(self, n):
        return jax.random.permutation(self._next(), n)


kernel_name = 'standalone__mha_softmax__decode'

def setup_inputs():
    _rng = _Rng(jax.random.key(int.from_bytes(__import__("os").urandom(4), "little")))
    _w = (lambda a: (lambda t: t.astype(jnp.bfloat16) if jnp.issubdtype(t.dtype, jnp.floating) else t)(jnp.asarray(a)))
    B, H, Sq, Sk, D = 1, 32, 1, 8192, 128
    return {
        "q": _w((lambda *s: _rng.normal(s) * 0.8)(B, H, Sq, D)),
        "k": _w((lambda *s: _rng.normal(s) * 0.8)(B, H, Sk, D)),
        "v": _w((lambda *s: _rng.normal(s) * 0.05)(B, H, Sk, D)),
    }

def reference(q, k, v):
    scale = q.shape[-1] ** -0.5
    scores = jnp.einsum("bhqd,bhkd->bhqk", q, k) * scale
    p = _softmax(scores, axis=-1)
    return jnp.einsum("bhqk,bhkd->bhqd", p, v)
```

```python
import jax, jax.numpy as jnp, numpy as np, functools
from jax import lax
from jax.experimental import pallas as pl
from jax.experimental.pallas import tpu as pltpu

def make_v1(depth=8, order=(3, 2, "r"), checks=False, flags=None, name=None):
    def fn(q, k, v):
        B, H, Sq, D = q.shape
        Sk = k.shape[2]
        T = 128
        NT = Sk // T
        NS = 2 * NT
        scale = D ** -0.5
        def kernel(q_hbm, k_hbm, v_hbm, o_hbm, buf, s_ref, q_v, o_v, sems, qsem):
            qc = pltpu.make_async_copy(q_hbm, q_v, qsem)
            def start(src, step, slot):
                hb = step // NT
                t = lax.rem(step, NT)
                for j in range(8):
                    bits = {order[b]: (j >> b) & 1 for b in range(3)}
                    for w in (1, 0):
                        hi = w * 4 + bits[3] * 2 + bits[2]
                        row = pl.multiple_of(t * T + bits["r"] * 64, 64)
                        pltpu.make_async_copy(src.at[hi, hb, :, pl.ds(row, 64)], buf.at[slot, hi, :, pl.ds(bits["r"] * 64, 64)],
                                              sems.at[slot]).start(priority=w)
            def wait(slot):
                pltpu.make_async_copy(buf.at[slot], buf.at[slot], sems.at[slot]).wait()
            nxt = lambda s: jnp.where(s + 1 == depth, 0, s + 1)
            sub = lax.broadcasted_iota(jnp.int32, (8, T), 0)

            start(k_hbm, 0, 0)
            qc.start()
            def pro(i, _):
                start(k_hbm, i, i)
            lax.fori_loop(1, depth, pro, None)
            qc.wait()
            qf = q_v[...].astype(jnp.float32)
            def qrows(hb, w):
                rows = [w * 16 + (r >> 1) * 4 + hb * 2 + (r & 1) for r in range(8)]
                return jnp.concatenate([qf[r:r + 1] for r in rows], axis=0).astype(jnp.bfloat16)

            def kstep(step, slot, qs, m):
                wait(slot)
                out = []
                for w in range(2):
                    s = None
                    for r in range(8):
                        x = lax.dot_general(qs[w], buf[slot, w * 4 + (r >> 1), r & 1], (((1,), (1,)), ((), ())),
                                            preferred_element_type=jnp.float32)
                        s = x if s is None else jnp.where(sub == r, x, s)
                    s = s * scale
                    s_ref[step, w] = s
                    out.append(jnp.maximum(m[w], s))
                return out
            def vstep(step, slot, mx, carry):
                l, acc = carry
                wait(slot)
                lo, ao = [], []
                for w in range(2):
                    p = jnp.exp(s_ref[step, w] - mx[w])
                    pb = p.astype(jnp.bfloat16)
                    o = None
                    for r in range(8):
                        x = jnp.dot(pb, buf[slot, w * 4 + (r >> 1), r & 1], preferred_element_type=jnp.float32)
                        o = x if o is None else jnp.where(sub == r, x, o)
                    lo.append(l[w] + p); ao.append(acc[w] + o)
                return lo, ao

            neg = jnp.full((8, T), -jnp.inf, jnp.float32)
            zero = jnp.zeros((8, T), jnp.float32)
            slot = 0
            mx = []
            for hb in range(2):
                qs = [qrows(hb, 0), qrows(hb, 1)]
                def body(step, c, src, off):
                    slot, m = c
                    m = kstep(step, slot, qs, m)
                    start(src, step + depth - off, slot)
                    return nxt(slot), m
                if hb == 0:
                    slot, m = lax.fori_loop(0, NT, functools.partial(body, src=k_hbm, off=0), (slot, [neg, neg]))
                else:
                    slot, m = lax.fori_loop(NT, NS - depth, functools.partial(body, src=k_hbm, off=0), (slot, [neg, neg]))
                    slot, m = lax.fori_loop(NS - depth, NS, functools.partial(body, src=v_hbm, off=NS), (slot, m))
                mx.append([jnp.broadcast_to(jnp.max(x, axis=1, keepdims=True), (8, T)) for x in m])
            for hb in range(2):
                def body(step, c, more):
                    slot, carry = c
                    carry = vstep(step, slot, mx[hb], carry)
                    if more: start(v_hbm, step + depth, slot)
                    return nxt(slot), carry
                init = ([zero, zero], [zero, zero])
                if hb == 0:
                    slot, (l, acc) = lax.fori_loop(0, NT, functools.partial(body, more=True), (slot, init))
                else:
                    slot, cr = lax.fori_loop(NT, NS - depth, functools.partial(body, more=True), (slot, init))
                    slot, (l, acc) = lax.fori_loop(NS - depth, NS, functools.partial(body, more=False), (slot, cr))
                for w in range(2):
                    o = acc[w] / jnp.sum(l[w], axis=1, keepdims=True)
                    for r in range(0, 8, 2):
                        o_v[pl.ds(w * 16 + (r >> 1) * 4 + hb * 2, 2), :] = o[r:r + 2]
            q_v[...] = o_v[...].astype(q_v.dtype)
            oc = pltpu.make_async_copy(q_v, o_hbm, qsem); oc.start(); oc.wait()
        out = pl.pallas_call(
            kernel,
            in_specs=[pl.BlockSpec(memory_space=pl.ANY)] * 3,
            out_specs=pl.BlockSpec(memory_space=pl.ANY),
            out_shape=jax.ShapeDtypeStruct((H, D), q.dtype),
            scratch_shapes=[pltpu.VMEM((depth, 8, 2, T, D), k.dtype), pltpu.VMEM((NS, 2, 8, T), jnp.float32),
                            pltpu.VMEM((H, D), q.dtype), pltpu.VMEM((H, D), jnp.float32),
                            pltpu.SemaphoreType.DMA((depth,)), pltpu.SemaphoreType.DMA(())],
            compiler_params=pltpu.CompilerParams(vmem_limit_bytes=64 * 2**20, disable_bounds_checks=not checks, flags=flags),
            name=name,
        )(q.reshape(H, D), k.reshape(8, 2, 2, Sk, D), v.reshape(8, 2, 2, Sk, D))
        return out.reshape(q.shape)
    return fn


@jax.jit
def pallas_standalone__mha_softmax__decode_kernel(q, k, v):
    return make_v1(8, checks=True)(q, k, v)
```

```python
import functools

import jax
import jax.numpy as jnp
from jax import lax
from jax.experimental import pallas as pl
from jax.experimental.pallas import tpu as pltpu

GROUP = 8
HALF = 64
TILE = 2 * HALF
ROWS = 2
SLOTS = 8

ISSUE = ((1, 0), (1, 1), (1, 2), (0, 5), (1, 3), (0, 6), (1, 4), (0, 7))
HEADS = tuple(tuple(h for p, h in ISSUE if p == prio) for prio in (0, 1))
WARMUP = tuple(0 if n % 16 == 1 else 1 for n in range(35))
DRAIN = 4
LAST_GROUPS = (5, 2, 2, 1)


def _attention_kernel(
    q_hbm, k_hbm, v_hbm, o_hbm, buf, s_ref, pt_ref, io_ref, q_ref, out_ref, *, scale
):
    n_heads, head_dim = q_hbm.shape
    n_groups = n_heads // GROUP
    n_steps = k_hbm.shape[2] // (ROWS * HALF)
    tiles = [[(r, h) for r in range(ROWS) for h in hs] for hs in HEADS]
    last_sem = dict(
        zip(tiles[1], (i for i, n in enumerate(LAST_GROUPS) for _ in range(n)), strict=True)
    )

    def run(io_sem, sems, last_sems):
        def copy(src, group, step, slot, r, h, sem):
            key = (step * ROWS + r) * HALF
            if not isinstance(key, int):
                key = pl.multiple_of(key, HALF)
            return pltpu.make_async_copy(
                src.at[group * GROUP + h, :, pl.ds(key, HALF)], buf.at[slot, r, h], sem
            )

        def start(src, group, step, slot, *, priorities=(), last=False):
            copies = [(r, prio, h) for r in range(ROWS) for prio, h in ISSUE]
            for n, (r, prio, h) in enumerate(copies):
                sem = last_sems.at[last_sem[r, h]] if last and prio else sems.at[prio, slot]
                copy(src, group, step, slot, r, h, sem).start(
                    priority=priorities[n] if n < len(priorities) else prio
                )

        def wait(slot, prio):
            part = buf.at[slot, :, pl.ds(HEADS[prio][0], len(HEADS[prio]))]
            pltpu.make_async_copy(part, part, sems.at[prio, slot]).wait()

        def tile(slot, r, h):
            return buf[slot, r, h].reshape(TILE, head_dim)

        def next_slot(slot):
            return jnp.where(slot + 1 == SLOTS, 0, slot + 1)

        def group_rows(group):
            row = group * GROUP
            return pl.ds(row if isinstance(row, int) else pl.multiple_of(row, GROUP), GROUP)

        def keep_row(h, x, rest):
            return jnp.where(lax.broadcasted_iota(jnp.int32, x.shape, 0) == h, x, rest)

        def add_pv(acc, p, slot, which):
            for r in range(ROWS):
                o = jnp.zeros_like(acc)
                for h in (h for rr, h in which if rr == r):
                    x = jnp.dot(
                        p[r].astype(buf.dtype),
                        tile(slot, r, h),
                        preferred_element_type=jnp.float32,
                    )
                    o = keep_row(h, x, o)
                acc += o
            return acc

        def score_pass(group, slot):
            q = q_ref[group_rows(group), :].astype(buf.dtype)

            def body(step, carry, src, ahead):
                slot, m = carry
                wait(slot, 0)
                wait(slot, 1)
                for r in range(ROWS):
                    s = jnp.zeros_like(m)
                    for h in range(GROUP):
                        x = lax.dot_general(
                            q,
                            tile(slot, r, h),
                            (((1,), (1,)), ((), ())),
                            preferred_element_type=jnp.float32,
                        )
                        s = keep_row(h, x, s)
                    s *= scale
                    s_ref[step * ROWS + r] = s
                    m = jnp.maximum(m, s)
                start(src, group, step + ahead, slot)
                return next_slot(slot), m

            carry = (slot, jnp.full((GROUP, TILE), -jnp.inf, jnp.float32))
            split = n_steps - SLOTS
            carry = lax.fori_loop(
                0, split, functools.partial(body, src=k_hbm, ahead=SLOTS), carry
            )
            slot, m = lax.fori_loop(
                split, n_steps, functools.partial(body, src=v_hbm, ahead=-split), carry
            )
            return slot, jnp.broadcast_to(jnp.max(m, axis=1, keepdims=True), m.shape)

        def exp_scores(step, m):
            return [jnp.exp(s_ref[step * ROWS + r] - m) for r in range(ROWS)]

        def value_step(step, carry, m, refill):
            slot, l, acc = carry
            wait(slot, 0)
            wait(slot, 1)
            p = exp_scores(step, m)
            acc = add_pv(acc, p, slot, [(r, h) for r in range(ROWS) for h in range(GROUP)])
            refill(step, slot)
            return next_slot(slot), l + sum(p[1:], p[0]), acc

        def value_steps(lo, hi, carry, m, refill):
            body = functools.partial(value_step, m=m, refill=refill)
            return lax.fori_loop(lo, hi, body, carry)

        zeros = (
            jnp.zeros((GROUP, TILE), jnp.float32),
            jnp.zeros((GROUP, head_dim), jnp.float32),
        )

        per_step = ROWS * GROUP
        n_warm = pl.cdiv(len(WARMUP), per_step)
        for step in range(n_warm):
            start(k_hbm, 0, step, step, priorities=WARMUP[step * per_step :])
        q_copy = pltpu.make_async_copy(q_hbm, io_ref, io_sem)
        q_copy.start()
        lax.fori_loop(n_warm, SLOTS, lambda step, _: start(k_hbm, 0, step, step), None)
        q_copy.wait()
        q_ref[...] = io_ref[...].astype(jnp.float32)

        def full_group(group, slot):
            slot, m = score_pass(group, slot)
            split = n_steps - SLOTS
            carry = value_steps(
                0, split, (slot, *zeros), m,
                lambda step, slot: start(v_hbm, group, step + SLOTS, slot),
            )
            slot, l, acc = value_steps(
                split, n_steps, carry, m,
                lambda step, slot: start(k_hbm, group + 1, step - split, slot),
            )
            out_ref[group_rows(group), :] = acc / jnp.sum(l, axis=1, keepdims=True)
            return slot

        group = n_groups - 1
        slot = lax.fori_loop(0, group, full_group, 0)

        slot, m = score_pass(group, slot)
        split = n_steps - SLOTS - 1
        carry = value_steps(
            0, split, (slot, *zeros), m,
            lambda step, slot: start(v_hbm, group, step + SLOTS, slot),
        )
        carry = value_step(
            split, carry, m,
            lambda step, slot: start(v_hbm, group, n_steps - 1, slot, last=True),
        )
        _, l, acc = value_steps(
            split + 1, n_steps - DRAIN, carry, m, lambda step, slot: None
        )
        p = [exp_scores(step, m) for step in range(n_steps - DRAIN, n_steps)]
        inv = 1.0 / jnp.sum(sum(sum(p, []), l), axis=1, keepdims=True)
        p = [[x * inv for x in ps] for ps in p]
        acc *= inv
        for n, (r, h) in enumerate(tiles[1]):
            pt_ref[n] = jnp.broadcast_to(p[-1][r][h : h + 1], (head_dim, TILE)).T
        slots = [(2 * n_groups * n_steps - DRAIN + i) % SLOTS for i in range(DRAIN)]
        for slot in slots:
            wait(slot, 0)
        for ps, slot in zip(p, slots):
            acc = add_pv(acc, ps, slot, tiles[0])
        for ps, slot in zip(p[:-1], slots[:-1]):
            wait(slot, 1)
            acc = add_pv(acc, ps, slot, tiles[1])
        for i in range(len(LAST_GROUPS)):
            arrived = [t for t in tiles[1] if last_sem[t] == i]
            for r, h in arrived:
                copy(v_hbm, group, n_steps - 1, slots[-1], r, h, last_sems.at[i]).wait()
            for r, h in arrived:
                x = tile(slots[-1], r, h).astype(jnp.float32) * pt_ref[tiles[1].index((r, h))]
                x = jnp.sum(x.reshape(4, TILE // 4, head_dim), axis=0)
                x = jnp.broadcast_to(jnp.sum(x, axis=0, keepdims=True), acc.shape)
                acc += keep_row(h, x, 0.0)

        done = out_ref[pl.ds(0, group * GROUP), :]
        io_ref[...] = jnp.concatenate([done, acc], axis=0).astype(io_ref.dtype)
        o_copy = pltpu.make_async_copy(io_ref, o_hbm, io_sem)
        o_copy.start()
        o_copy.wait()

    pl.run_scoped(
        run,
        pltpu.SemaphoreType.DMA(()),
        pltpu.SemaphoreType.DMA((2, SLOTS)),
        pltpu.SemaphoreType.DMA((len(LAST_GROUPS),)),
    )


@jax.jit
def pallas_standalone__mha_softmax__decode_kernel(
    q: jax.Array,
    k: jax.Array,
    v: jax.Array,
):
    batch, heads_per_batch, q_len, head_dim = q.shape
    n_keys = k.shape[2]
    n_heads = batch * heads_per_batch
    assert q_len == 1 and k.shape == v.shape and q.dtype == k.dtype == v.dtype
    assert n_heads % (2 * GROUP) == 0 and head_dim % 128 == 0
    assert n_keys % (ROWS * TILE) == 0 and n_keys // (ROWS * TILE) > SLOTS

    halves = (n_heads, 2, n_keys // 2, head_dim)
    out = pl.pallas_call(
        functools.partial(_attention_kernel, scale=head_dim**-0.5),
        in_specs=[pl.BlockSpec(memory_space=pl.ANY)] * 3,
        out_specs=pl.BlockSpec(memory_space=pl.ANY),
        out_shape=jax.ShapeDtypeStruct((n_heads, head_dim), q.dtype),
        scratch_shapes=[
            pltpu.VMEM((SLOTS, ROWS, GROUP, 2, HALF, head_dim), k.dtype),
            pltpu.VMEM((n_keys // TILE, GROUP, TILE), jnp.float32),
            pltpu.VMEM((sum(LAST_GROUPS), TILE, head_dim), jnp.float32),
            pltpu.VMEM((n_heads, head_dim), q.dtype),
            pltpu.VMEM((n_heads, head_dim), jnp.float32),
            pltpu.VMEM((n_heads - GROUP, head_dim), jnp.float32),
        ],
        name="mha_softmax_decode",
    )(q.reshape(n_heads, head_dim), k.reshape(halves), v.reshape(halves))
    return out.reshape(q.shape)
```
